```python
import os as _os
_os.environ.setdefault("JAX_PLATFORMS", "cpu")
import jax
import jax.numpy as jnp

def _softmax(x, axis=-1):
    return jax.nn.softmax(x, axis=axis)
def _gelu(x):
    return jax.nn.gelu(x, approximate=True)
def _silu(x):
    return jax.nn.silu(x)
def _sigmoid(x):
    return jax.nn.sigmoid(x)
def _layernorm(x, axis=-1, eps=1e-5):
    m = jnp.mean(x, axis=axis, keepdims=True)
    v = jnp.var(x, axis=axis, keepdims=True)
    return (x - m) / jnp.sqrt(v + eps)
def _scatter_add(tgt, idx, src, axis=0):
    return tgt.at[idx].add(src)
def _segment_sum(src, seg, n):
    return jax.ops.segment_sum(src, seg, n)
class _Rng:
    def __init__(self, key):
        self._k = key
    def _next(self):
        self._k, sub = jax.random.split(self._k)
        return sub
    def normal(self, shape):
        return jax.random.normal(self._next(), shape, dtype=jnp.bfloat16)
    def randint(self, lo, hi, shape):
        return jax.random.randint(self._next(), shape, lo, hi, dtype=jnp.int32)
    def uniform(self, shape, lo=0.0, hi=1.0):
        return jax.random.uniform(self._next(), shape, jnp.bfloat16, lo, hi)
    def permutation(self, n):
        return jax.random.permutation(self._next(), n)


kernel_name = 'concat_heads__mha_block_cached__mha_block_cached__near_ridge'

def setup_inputs():
    _rng = _Rng(jax.random.key(int.from_bytes(__import__("os").urandom(4), "little")))
    _w = (lambda a: (lambda t: t.astype(jnp.bfloat16) if jnp.issubdtype(t.dtype, jnp.floating) else t)(jnp.asarray(a)))
    def _A_setup():
        B, Sq, D = 16, 80, 512
        H, Sk, Dh = 32, 80, 128
        return {
            "x": _w((lambda *s: _rng.normal(s) * 0.8)(B, Sq, D)),
            "k_cache": _w((lambda *s: _rng.normal(s) * 0.8)(B, H, Sk, Dh)),
            "v_cache": _w((lambda *s: _rng.normal(s) * 0.05)(B, H, Sk, Dh)),
            "wq": _w((lambda *s: _rng.normal(s) * 0.8)(D, H * Dh) * (D ** -0.5)),
            "wo": _w((lambda *s: _rng.normal(s) * 0.05)(H * Dh, D) * ((H * Dh) ** -0.5)),
        }
    _A_in = _A_setup()

    def _B_setup():
        B, Sq, D = 16, 80, 512
        H, Sk, Dh = 32, 80, 128
        return {
            "x": _w((lambda *s: _rng.normal(s) * 0.8)(B, Sq, D)),
            "k_cache": _w((lambda *s: _rng.normal(s) * 0.8)(B, H, Sk, Dh)),
            "v_cache": _w((lambda *s: _rng.normal(s) * 0.05)(B, H, Sk, Dh)),
            "wq": _w((lambda *s: _rng.normal(s) * 0.8)(D, H * Dh) * (D ** -0.5)),
            "wo": _w((lambda *s: _rng.normal(s) * 0.05)(H * Dh, D) * ((H * Dh) ** -0.5)),
        }
    _B_in = _B_setup()

    return {
        "A_x": _A_in["x"],
        "A_k_cache": _A_in["k_cache"],
        "A_v_cache": _A_in["v_cache"],
        "A_wq": _A_in["wq"],
        "A_wo": _A_in["wo"],
        "B_x": _B_in["x"],
        "B_k_cache": _B_in["k_cache"],
        "B_v_cache": _B_in["v_cache"],
        "B_wq": _B_in["wq"],
        "B_wo": _B_in["wo"],
    }

def reference(A_x, A_k_cache, A_v_cache, A_wq, A_wo, B_x, B_k_cache, B_v_cache, B_wq, B_wo):
    def _A_ref(x, k_cache, v_cache, wq, wo):
        B, Sq, D = x.shape
        H, Dh = 32, 128
        q = (lambda x, *d: x.transpose(*d))((x @ wq).reshape(B, Sq, H, Dh), 0, 2, 1, 3)
        scores = jnp.einsum("bhqd,bhkd->bhqk", q, k_cache) * (Dh ** -0.5)
        p = _softmax(scores, axis=-1)
        o = jnp.einsum("bhqk,bhkd->bhqd", p, v_cache)
        return (lambda x, *d: x.transpose(*d))(o, 0, 2, 1, 3).reshape(B, Sq, H * Dh) @ wo

    def _B_ref(x, k_cache, v_cache, wq, wo):
        B, Sq, D = x.shape
        H, Dh = 32, 128
        q = (lambda x, *d: x.transpose(*d))((x @ wq).reshape(B, Sq, H, Dh), 0, 2, 1, 3)
        scores = jnp.einsum("bhqd,bhkd->bhqk", q, k_cache) * (Dh ** -0.5)
        p = _softmax(scores, axis=-1)
        o = jnp.einsum("bhqk,bhkd->bhqd", p, v_cache)
        return (lambda x, *d: x.transpose(*d))(o, 0, 2, 1, 3).reshape(B, Sq, H * Dh) @ wo

    a = _A_ref(A_x, A_k_cache, A_v_cache, A_wq, A_wo)
    b = _B_ref(B_x, B_k_cache, B_v_cache, B_wq, B_wo)
    return jnp.concatenate([a, b], axis=-1)
```

```python
import math
import jax, jax.numpy as jnp
import jax.experimental.pallas as pl
import jax.experimental.pallas.tpu as pltpu

B,SQ,D,H,SK,DH = 16,80,512,32,80,128
NB,NH=4,4
NJ,NG=B//NB,H//NH
NT_=2*NG*NJ
MS=NB*SQ
F32,BF16,U32=jnp.float32,jnp.bfloat16,jnp.uint32
def pk2(a,b): return pltpu.pack_elementwise([a,b],packed_dtype=BF16)
def pk(x): return pk2(x[0:8],x[8:16])
def un(x,i): return pltpu.unpack_elementwise(x,index=i,packed_dtype=BF16,unpacked_dtype=F32)
def up(x): return pltpu.bitcast(x,BF16)
C2=DH**-0.5*math.log2(math.e)
NT=(((1,),(1,)),((),()))

def quad(m):
    n=len(m)//2
    return ([r[:n] for r in m[:n]],[r[n:] for r in m[:n]],[r[:n] for r in m[n:]],[r[n:] for r in m[n:]])
def madd(a,b): return [[x+y for x,y in zip(r,s)] for r,s in zip(a,b)]
def msub(a,b): return [[x-y for x,y in zip(r,s)] for r,s in zip(a,b)]
def lhs_terms(m,lv):
    if lv==0: return [m]
    a11,a12,a21,a22=quad(m)
    return [t for s in (madd(a11,a22),madd(a21,a22),a11,a22,madd(a11,a12),msub(a21,a11),msub(a12,a22)) for t in lhs_terms(s,lv-1)]
def rhs_terms(m,lv):
    if lv==0: return [m]
    b11,b12,b21,b22=quad(m)
    return [t for s in (madd(b11,b22),b11,msub(b12,b22),msub(b21,b11),b22,madd(b11,b12),madd(b21,b22)) for t in rhs_terms(s,lv-1)]
def combine(ps,lv):
    if lv==0: return ps[0]
    n=len(ps)//7
    m1,m2,m3,m4,m5,m6,m7=[combine(ps[i*n:(i+1)*n],lv-1) for i in range(7)]
    c11=madd(madd(m1,m4),msub(m7,m5)); c12=madd(m3,m5); c21=madd(m2,m4); c22=madd(msub(m1,m2),madd(m3,m6))
    return [a+b for a,b in zip(c11,c12)]+[a+b for a,b in zip(c21,c22)]

LT=[((0,1),(3,1)),((2,1),(3,1)),((0,1),),((3,1),),((0,1),(1,1)),((2,1),(0,-1)),((1,1),(3,-1))]
RT=[((0,1),(3,1)),((0,1),),((1,1),(3,-1)),((2,1),(0,-1)),((3,1),),((0,1),(1,1)),((2,1),(3,1))]
WT=[((0,1),(3,1),(4,-1),(6,1)),((2,1),(4,1)),((1,1),(3,1)),((0,1),(1,-1),(2,1),(5,1))]
def lin(terms,get):
    y=None
    for q,sg in terms:
        v=get(q); y=v if y is None else (y+v if sg>0 else y-v)
    return y
def interleave(*lists):
    items=[]
    for k,(l,lo,hi) in enumerate(lists):
        for i,t in enumerate(l): items.append((lo+(hi-lo)*(i+0.5)/len(l),k,i,t))
    return [t for *_,t in sorted(items,key=lambda z:z[:3])]

def build(qr=(0.051,0.975),orr=(0.001,0.998),kr=(0.065,0.739),lag=0.271,kt=(0.0,0.6),lt=0.4,qs=0.529,jr=(0.013,0.896),QO=(1,0,2,3),qtv=1,fuse=0,cut=1,kv1=0,pw=1,early=1,rolls=0,t0=0,dq_=0,Q4=0,quick=0,bc=0,stg=1,nit=NG,flags=None,off=''):
    R=49; NGG=2*NG
    def kern(xa,ka,va,wqa,woa,xb,kb,vb,wqb,wob,out,
             xs,xc,wqs,wos,wqc,woc,ks,vs,qt,qc,os_,acc,ob,xsem,wqsem,wosem,kvsem,kv0sem,osem):
        def ds(i,n): return pl.ds(i,n) if isinstance(i,int) else pl.ds(pl.multiple_of(i,n),n)
        def both(gg,fn):
            if 'm' in off: return
            if isinstance(gg,int):
                if gg<NGG: fn(gg//NG,gg%NG)
                return
            @pl.when(gg<NG)
            def _(): fn(0,gg)
            @pl.when((gg>=NG)&(gg<NGG))
            def _(): fn(1,gg-NG)
        def x_copy(br,j): return pltpu.make_async_copy((xa,xb)[br].at[ds(j*MS,MS),:],xs.at[br,j],xsem.at[br*NJ+j])
        def wq_copy(br,g,sl): return pltpu.make_async_copy((wqa,wqb)[br].at[:,ds(g*512,512)],wqs.at[sl],wqsem.at[sl])
        def wo_copy(br,g,sl): return pltpu.make_async_copy((woa,wob)[br].at[ds(g*512,512),:],wos.at[sl],wosem.at[sl])
        def kv_copy(c,br,g,sl,h): return pltpu.make_async_copy(((ka,kb),(va,vb))[c][br].at[pl.ds(h*cut*NB,(cut,NJ-cut)[h]*NB),pl.ds(g*NH,NH)],(ks,vs)[c].at[sl,pl.ds(h*cut*NB,(cut,NJ-cut)[h]*NB)],kvsem.at[h*4+c*2+sl])
        def kv0_copy(c,j): return pltpu.make_async_copy((ka,va)[c].at[pl.ds(j*NB,NB),pl.ds(0,NH)],(ks,vs)[c].at[0,pl.ds(j*NB,NB)],kv0sem.at[c*NJ+j])
        def o_copy(br,j): return pltpu.make_async_copy(ob.at[j],out.at[ds(j*MS,MS),pl.ds(br*D,D)],osem.at[j])
        def start_kv(gg,sl,hs=(0,1)): both(gg,lambda br,g: [kv_copy(c,br,g,sl,h).start() for h in hs for c in range(2)] and None)
        def exists(gg,fn):
            if 'm' in off: return
            if isinstance(gg,int): fn()
            else: pl.when(gg<NGG)(fn)
        def wait_kv(sl,hs=(0,1)): exists(0,lambda: [kv_copy(c,0,0,sl,h).wait() for h in hs for c in range(2)])
        def start_kv0(j): exists(0,lambda: [kv0_copy(c,j).start() for c in range(2)])
        def wait_kv0(j): exists(0,lambda: [kv0_copy(c,j).wait() for c in range(2)])
        def start_w(cp,gg,sl): both(gg,lambda br,g: cp(br,g,sl).start())
        def wait_w(cp,gg,sl): exists(gg,lambda: cp(0,0,sl).wait())
        def words(raw,sl,r,c):
            if bc&1: return raw.bitcast(U32)[sl,ds(r//2,8),c:c+128]
            return pltpu.bitcast(raw[sl,ds(r,16),c:c+128],U32)
        def tile(ref,sl,j,u): return up(ref.bitcast(U32)[sl,j*NB+u//4,u%4]) if bc&2 else ref[sl,j*NB+u//4,u%4]
        def x_jobs(br,j):
            def job(r0,i):
                blk=[[lin(LT[i],lambda q: xs[br,j,(2*(q//2)+a)*SQ+r0:(2*(q//2)+a)*SQ+r0+16,(2*(q%2)+b)*128:(2*(q%2)+b+1)*128].astype(F32)) for b in range(2)] for a in range(2)]
                ys=[pk(t[0][0]) for t in lhs_terms(blk,1)]
                for k in range(7): xc[j,i*7+k,r0//2:r0//2+8,:]=ys[k]
                return ys
            return [(lambda r0=r0,i=i: job(r0,i)) for i in range(7) for r0 in range(0,SQ,16)]
        def w_job(raw,dst,sl,r0,i):
            u=[rhs_terms([[lin(RT[i],lambda q: un(words(raw,sl,(2*(q//2)+a)*128+r0,(2*(q%2)+b)*128),k)) for b in range(2)] for a in range(2)],1) for k in range(2)]
            ys=[pk2(u[0][k][0][0],u[1][k][0][0]) for k in range(7)]
            for k in range(7): dst[sl,i*7+k,ds(r0//2,8),:]=ys[k]
            return ys
        def w_jobs(raw,dst,sl,j): return [(lambda k=k,i=i: w_job(raw,dst,sl,j*32+k*16,i)) for k in range(2) for i in range(7)]
        def full_w(raw,dst,sl):
            @pl.loop(0,8)
            def _(k):
                for i in range(7): w_job(raw,dst,sl,k*16,i)
        def fin_jobs(j):
            def job(r0,Q):
                c=[combine([[[lin(WT[Q],lambda m: acc[j,m*7+k,r:r+8,:])]] for k in range(7)],1) for r in (r0,r0+8)]
                ys=[]
                for a in range(2):
                    for b in range(2):
                        rr=(2*(Q//2)+a)*SQ+r0; cc=(2*(Q%2)+b)*128
                        ys.append(pk2(c[0][a][b],c[1][a][b])); ob[j,rr:rr+16,cc:cc+128]=up(ys[-1])
                return ys
            return [(lambda r0=r0,Q=Q: job(r0,Q)) for r0 in range(0,SQ,16) for Q in range(4)]
        def half(par,j,never,dq=True,da=True,do=True,wq=True,wo=True,first=False,extra=(),cnt0=0):
            pend=[]
            def tie(vs_):
                vs_=list(vs_)
                for t in range(t0,len(vs_)):
                    if pend: vs_[t]=jnp.where(never,pend.pop(0),vs_[t])
                return up(jnp.concatenate(vs_,axis=0))
            items=[]; jobs=list(extra)
            def add(fs,n,lo,hi):
                for t,f in enumerate(fs): items.append((lo+(hi-lo)*(t+0.5)/len(fs),len(items),n,f))
            unit=lambda Q,k: (2*(Q//2)+k//2)*4+2*(Q%2)+k%2
            if da:
                sl=par; e=[None]*16
                qv={}
                def qprep(Q,k):
                    cs=[lin(WT[Q],lambda i: qc[par,j,i*4+k,r:r+8,:]) for r in range(0,SQ,8)]
                    qv[Q,k]=[pk2(cs[t],cs[t+1]) for t in range(0,10,2)]
                    if dq_: pend[:0]=qv[Q,k]
                def qk(Q,k):
                    u=unit(Q,k)
                    q=up(jnp.concatenate(qv[Q,k],axis=0))
                    sc=jax.lax.dot_general(tile(ks,sl,j,u),q,NT,preferred_element_type=F32)
                    z=jnp.exp2((sc-jnp.max(sc,axis=0,keepdims=True))*C2)
                    l=jnp.sum(z,axis=0,keepdims=True)
                    y=pl.reciprocal(l,approx=True); r=y*(2.0-l*y)
                    e[u]=(z*r).astype(BF16).T
                def pv(k):
                    o=[jnp.dot(e[unit(Q,k)],tile(vs,sl,j,unit(Q,k)),preferred_element_type=F32) for Q in range(4)]
                    for i in range(7): os_[par,j,i*4+k]=lin(LT[i],lambda Q: o[Q])
                k0,k1,lg=(*kr,lag) if (dq and do) else (*kt,lt)
                add([(lambda Q=Q,k=k: qprep(Q,k)) for k in range(4) for Q in QO],0,k0-dq_,k1-dq_)
                add([(lambda Q=Q,k=k: qk(Q,k)) for k in range(4) for Q in QO],1,k0,k1)
                add([(lambda k=k: pv(k)) for k in range(4)],4,k0+lg,k1+lg)
            if dq:
                slq,jq=1-par,j; tmp={}
                def qd(p): return jnp.dot(tie([xc[jq,p,t:t+8,:] for t in range(0,SQ//2,8)]),up(wqc[slq,p]),preferred_element_type=F32)
                def q3(i,m):
                    if qtv: tmp[i,m]=qd(i*7+m)
                    else: qt[i*3+(1,2,5).index(m)]=qd(i*7+m)
                def q4(i):
                    ms={m:qd(i*7+m) for m in (0,3,4,6)}
                    for k in range(4): qc[1-par,j,i*4+k]=lin(WT[k],lambda m: ms[m] if m in ms else tmp[i,m] if qtv else qt[i*3+(1,2,5).index(m)])
                w=(qr[1]-qr[0])/7
                for i in range(7):
                    add([(lambda m=m,i=i: q3(i,m)) for m in (1,2,5)],1,qr[0]+w*(i-qs),qr[0]+w*(i+0.6-qs))
                    add([lambda i=i: q4(i)],4,qr[0]+w*(i+0.8),qr[0]+w*(i+0.8))
                if wq and 'w' not in off: jobs+=w_jobs(wqs,wqc,1-slq,jq)
            if do:
                slo,jo=1-par,j
                def od(p):
                    cs=[lin(LT[p%7],lambda k: os_[1-par,j,(p//7)*4+k,t:t+8,:]) for t in range(0,SQ,8)]
                    y=jnp.dot(tie([pk2(cs[t],cs[t+1]) for t in range(0,10,2)]),up(woc[slo,p]),preferred_element_type=F32)
                    if first is True: acc[jo,p]=y
                    elif first is False: acc[jo,p]+=y
                    else: acc[jo,p]=jnp.where(first,0.0,acc[jo,p])+y
                add([(lambda p=p: od(p)) for p in range(R)],1,*orr)
                if wo and 'w' not in off: jobs+=w_jobs(wos,woc,1-slo,jo)
            if jobs: add([(lambda f=f: pend.extend(f())) for f in jobs],0,*jr)
            cnt=cnt0; held=[]
            for _,_,n,f in sorted(items,key=lambda z:z[:2]):
                if n==4: held.append(f)
                else: f(); cnt+=n
                while held and cnt%4==0: held.pop(0)(); cnt+=4
            for f in held: f(); cnt+=4
            return cnt
        if quick:
            @pl.loop(0,nit)
            def _(i):
                wq_copy(0,0,0).start(); wq_copy(0,0,1).start(); wo_copy(0,0,0).start(); wo_copy(0,0,1).start()
                wq_copy(0,0,0).wait(); wq_copy(0,0,1).wait(); wo_copy(0,0,0).wait(); wo_copy(0,0,1).wait()
                c=0
                for j in range(quick):
                    c=half(1,j,i<0,cnt0=c)
            for f in fin_jobs(3): f()
            o_copy(1,3).start(); o_copy(1,3).wait()
            return
        def run(jobs):
            for f in jobs: f()
        def slices(roll,fn):
            if roll: pl.loop(0,NJ)(lambda j: fn(j,j<0,0) and None)
            else:
                c=0
                for j in range(NJ): c=fn(j,never0,c)
        never0=pl.program_id(0)>0
        x_copy(0,0).start(); start_w(wq_copy,0,0)
        x_copy(0,0).wait()
        x_copy(0,1).start(); x_copy(0,2).start()
        run(x_jobs(0,0))
        wait_w(wq_copy,0,0)
        x_copy(0,3).start(); start_w(wq_copy,1,1); start_kv0(0)
        full_w(wqs,wqc,0)
        start_w(wq_copy,2,0); start_w(wo_copy,0,0)
        def head0(j,never,c):
            half(1,j,never,da=False,do=False,wq=False)
            @pl.when(j<NJ-1)
            def _():
                x_copy(0,j+1).wait(); start_kv0(j+1); run(x_jobs(0,j+1))
        slices(True,head0)
        if early: start_kv(1,1,range(early))
        wait_w(wq_copy,1,1); full_w(wqs,wqc,1)
        wait_w(wq_copy,2,0); wait_w(wo_copy,0,0)
        def quad(par,never,extra=lambda j: (),pre=None,post=None,**kw):
            c=0
            for j in range(NJ):
                if pre: pre(j)
                c=half(par,j,never,extra=extra(j),cnt0=c,**kw)
                if post: post(j)
        if rolls&1:
            start_kv(1,1); start_w(wq_copy,3,1); start_w(wo_copy,1,1)
            def head1(j,never,c):
                wait_kv0(j)
                return half(0,j,never,do=False,extra=w_jobs(wos,woc,0,j),cnt0=c)
            slices(True,head1)
            start_w(wq_copy,4,0); start_w(wo_copy,2,0); start_kv(2,0)
        @pl.loop(rolls&1,NGG+1)
        def _(g):
            never=g<0
            if not rolls&1:
                @pl.when(g==0)
                def _():
                    start_w(wq_copy,3,1); start_w(wo_copy,1,1)
                    if early<1: start_kv(1,1,(0,))
                    def pre(j):
                        if j%pw==0:
                            for t in range(j,j+pw): wait_kv0(t)
                        if j==kv1 and early<2: start_kv(1,1,(1,))
                    quad(0,never,extra=lambda j: w_jobs(wos,woc,0,j),pre=pre,do=False)
                    start_w(wq_copy,4,0); start_w(wo_copy,2,0); start_kv(2,0)
            @pl.when(g==3)
            def _():
                for j in range(NJ): x_copy(1,j).start()
            @pl.when(g==NG-2)
            def _():
                for j in range(NJ): x_copy(1,j).wait()
            @pl.when(g==NG-1)
            def _():
                if fuse&1: run(x_jobs(1,NJ-1))
                else: pl.loop(0,NJ)(lambda j: run(x_jobs(1,j)))
            @pl.when(g==NG+1)
            def _():
                if fuse&2: run(fin_jobs(0))
                else: pl.loop(0,NJ)(lambda j: run(fin_jobs(j)))
            for par,first in ((0,False),(1,True),(1,False)):
                cond=(g%2==par)&(g>0)&(g<NGG-1)
                if par: cond=cond&((g%NG==1) if first else (g%NG!=1))
                @pl.when(cond)
                def _():
                    wait_w(wq_copy,g+2,par); wait_w(wo_copy,g,par); wait_kv(par,(0,) if first else (0,1))
                    quad(par,never,first=first,pre=lambda j: wait_kv(par,(1,)) if (first and j==cut) else None)
                    start_w(wq_copy,g+4,par); start_w(wo_copy,g+2,par); start_kv(g+2,par)
            @pl.when(g==NG+1)
            def _():
                for j in range(NJ): o_copy(0,j).start()
            @pl.when(g==NG+2)
            def _():
                for j in range(NJ): o_copy(0,j).wait()
            @pl.when(g==NGG-1)
            def _():
                wait_w(wo_copy,NGG-1,1); wait_kv(1)
                quad(1,never,dq=False)
            @pl.when(g==NGG)
            def _():
                quad(0,never,dq=False,da=False,wo=False,extra=lambda j: fin_jobs(j-1) if j else (),post=lambda j: o_copy(1,j-1).start() if j else None)
                run(fin_jobs(NJ-1)); o_copy(1,NJ-1).start()
        for j in range(NJ): o_copy(1,j).wait()

    def f(ax,ak,av,awq,awo,bx,bk,bv,bwq,bwo):
        V=pltpu.VMEM; S=pltpu.SemaphoreType.DMA
        out=pl.pallas_call(kern,grid=(1,),in_specs=[pl.BlockSpec(memory_space=pl.ANY)]*10,
            out_specs=pl.BlockSpec(memory_space=pl.ANY),
            out_shape=jax.ShapeDtypeStruct((B*SQ,2*D),BF16),
            scratch_shapes=[V((2,NJ,MS,D),BF16),V((NJ,R,SQ//2,128),U32),V((2,512,512),BF16),V((2,512,512),BF16),
                V((2,R,64,128),U32),V((2,R,64,128),U32),
                V((2,B,NH,SK,DH),BF16),V((2,B,NH,SK,DH),BF16),
                V((21,SQ,128),F32),V((2,NJ,28,SQ,128),F32),V((2,NJ,28,SQ,DH),F32),V((NJ,R,SQ,128),F32),V((NJ,MS,D),BF16),
                S((2*NJ,)),S((2,)),S((2,)),S((8,)),S((2*NJ,)),S((NJ,))],
            compiler_params=pltpu.CompilerParams(vmem_limit_bytes=100*2**20,flags=({k:True for k in flags.split('+')} if flags else None)),
        )(ax.reshape(B*SQ,D),ak,av,awq,awo,bx.reshape(B*SQ,D),bk,bv,bwq,bwo)
        return out.reshape(B,SQ,2*D)
    return f


@jax.jit
def pallas_concat_heads__mha_block_cached__mha_block_cached__near_ridge_kernel(
    A_x, A_k_cache, A_v_cache, A_wq, A_wo, B_x, B_k_cache, B_v_cache, B_wq, B_wo):
    return build()(A_x, A_k_cache, A_v_cache, A_wq, A_wo, B_x, B_k_cache, B_v_cache, B_wq, B_wo)
```

```python
import math
import jax, jax.numpy as jnp
import jax.experimental.pallas as pl
import jax.experimental.pallas.tpu as pltpu

B,SQ,D,H,SK,DH = 16,80,512,32,80,128
NB,NH=4,4
NJ,NG=B//NB,H//NH
NT_=2*NG*NJ
MS=NB*SQ
F32,BF16,U32=jnp.float32,jnp.bfloat16,jnp.uint32
def pk2(a,b): return pltpu.pack_elementwise([a,b],packed_dtype=BF16)
def pk(x): return pk2(x[0:8],x[8:16])
def un(x,i): return pltpu.unpack_elementwise(x,index=i,packed_dtype=BF16,unpacked_dtype=F32)
def up(x): return pltpu.bitcast(x,BF16)
C2=DH**-0.5*math.log2(math.e)
NT=(((1,),(1,)),((),()))

def quad(m):
    n=len(m)//2
    return ([r[:n] for r in m[:n]],[r[n:] for r in m[:n]],[r[:n] for r in m[n:]],[r[n:] for r in m[n:]])
def madd(a,b): return [[x+y for x,y in zip(r,s)] for r,s in zip(a,b)]
def msub(a,b): return [[x-y for x,y in zip(r,s)] for r,s in zip(a,b)]
def lhs_terms(m,lv):
    if lv==0: return [m]
    a11,a12,a21,a22=quad(m)
    return [t for s in (madd(a11,a22),madd(a21,a22),a11,a22,madd(a11,a12),msub(a21,a11),msub(a12,a22)) for t in lhs_terms(s,lv-1)]
def rhs_terms(m,lv):
    if lv==0: return [m]
    b11,b12,b21,b22=quad(m)
    return [t for s in (madd(b11,b22),b11,msub(b12,b22),msub(b21,b11),b22,madd(b11,b12),madd(b21,b22)) for t in rhs_terms(s,lv-1)]
LT=[((0,1),(3,1)),((2,1),(3,1)),((0,1),),((3,1),),((0,1),(1,1)),((2,1),(0,-1)),((1,1),(3,-1))]
RT=[((0,1),(3,1)),((0,1),),((1,1),(3,-1)),((2,1),(0,-1)),((3,1),),((0,1),(1,1)),((2,1),(3,1))]
WT=[((0,1),(3,1),(4,-1),(6,1)),((2,1),(4,1)),((1,1),(3,1)),((0,1),(1,-1),(2,1),(5,1))]
FLIP=(0,0,1,0,1,1,1)
def lin(terms,get):
    y=None
    for q,sg in terms:
        v=get(q); y=v if y is None else (y+v if sg>0 else y-v)
    return y
R=49
NGG=2*NG
CUT=1
T_QP,T_OP,T_QK,T_PV,T_JOB=(0.027,0.989),(0.016,1.017),(0.08,0.764),0.272,(0.008,0.86)
T_QLEAD,T_QK_SHORT,T_PV_SHORT=0.544,(0.024,0.607),0.376
QO=(1,0,2,3)


def build():
    def kern(xa,ka,va,wqa,woa,xb,kb,vb,wqb,wob,out,
             xs,xc,wqs,wos,wqc,woc,ks,vs,qc,os_,acc,ob,xsem,wqsem,wosem,kvsem,kv0sem,osem):
        def ds(i,n): return pl.ds(i,n) if isinstance(i,int) else pl.ds(pl.multiple_of(i,n),n)
        def both(gg,fn):
            if isinstance(gg,int):
                if gg<NGG: fn(gg//NG,gg%NG)
                return
            @pl.when(gg<NG)
            def _(): fn(0,gg)
            @pl.when((gg>=NG)&(gg<NGG))
            def _(): fn(1,gg-NG)
        def x_copy(br,j): return pltpu.make_async_copy((xa,xb)[br].at[ds(j*MS,MS),:],xs.at[br,j],xsem.at[br*NJ+j])
        def wq_copy(br,g,sl): return pltpu.make_async_copy((wqa,wqb)[br].at[:,ds(g*512,512)],wqs.at[sl],wqsem.at[sl])
        def wo_copy(br,g,sl): return pltpu.make_async_copy((woa,wob)[br].at[ds(g*512,512),:],wos.at[sl],wosem.at[sl])
        def kv_copy(c,br,g,sl,h):
            rows=pl.ds(h*CUT*NB,(CUT,NJ-CUT)[h]*NB) if sl else pl.ds(0,B)
            return pltpu.make_async_copy(((ka,kb),(va,vb))[c][br].at[rows,pl.ds(g*NH,NH)],(ks,vs)[c].at[sl,rows],kvsem.at[h*4+c*2+sl])
        def kv0_copy(c,j): return pltpu.make_async_copy((ka,va)[c].at[pl.ds(j*NB,NB),pl.ds(0,NH)],(ks,vs)[c].at[0,pl.ds(j*NB,NB)],kv0sem.at[c*NJ+j])
        def o_copy(br,j): return pltpu.make_async_copy(ob.at[j],out.at[ds(j*MS,MS),pl.ds(br*D,D)],osem.at[j])
        def start_kv(gg,sl,hs=(0,1)): both(gg,lambda br,g: [kv_copy(c,br,g,sl,h).start() for h in hs if h<=sl for c in range(2)] and None)
        def wait_kv(sl,hs=(0,1)):
            for h in hs:
                if h<=sl:
                    for c in range(2): kv_copy(c,0,0,sl,h).wait()
        def start_kv0(j):
            for c in range(2): kv0_copy(c,j).start()
        def wait_kv0(j):
            for c in range(2): kv0_copy(c,j).wait()
        def start_w(cp,gg,sl): both(gg,lambda br,g: cp(br,g,sl).start())
        def wait_w(cp,gg,sl):
            if isinstance(gg,int): cp(0,0,sl).wait()
            else: pl.when(gg<NGG)(lambda: cp(0,0,sl).wait())
        def words(raw,sl,r,c): return pltpu.bitcast(raw[sl,ds(r,16),c:c+128],U32)
        def tile(ref,sl,j,u): return ref[sl,j*NB+u//4,u%4]
        def x_jobs(br,j):
            def job(r0,i):
                blk=[[lin(LT[i],lambda q: xs[br,j,(2*(q//2)+a)*SQ+r0:(2*(q//2)+a)*SQ+r0+16,(2*(q%2)+b)*128:(2*(q%2)+b+1)*128].astype(F32)) for b in range(2)] for a in range(2)]
                ys=[pk(t[0][0]) for t in lhs_terms(blk,1)]
                for k in range(7): xc[j,i*7+k,r0//2:r0//2+8,:]=ys[k]
                return ys
            return [(lambda r0=r0,i=i: job(r0,i)) for i in range(7) for r0 in range(0,SQ,16)]
        def w_job(raw,dst,sl,r0,i):
            u=[rhs_terms([[lin(RT[i],lambda q: un(words(raw,sl,(2*(q//2)+a)*128+r0,(2*(q%2)+(b^FLIP[i]))*128),k)) for b in range(2)] for a in range(2)],1) for k in range(2)]
            ys=[pk2(u[0][k][0][0],u[1][k][0][0]) for k in range(7)]
            for k in range(7): dst[sl,i*7+k,ds(r0//2,8),:]=ys[k]
            return ys
        def w_jobs(raw,dst,sl,j): return [(lambda k=k,i=i: w_job(raw,dst,sl,j*32+k*16,i)) for k in range(2) for i in range(7)]
        def full_w(raw,dst,sl):
            @pl.loop(0,8)
            def _(k):
                for i in range(7): w_job(raw,dst,sl,k*16,i)
        def fin_jobs(j):
            def job(r0,Q):
                def rows(r):
                    out=[None]*4
                    for fl in (0,1):
                        tm=[t for t in WT[Q] if FLIP[t[0]]==fl]
                        if not tm: continue
                        tm.sort(key=lambda t:-t[1])
                        ps=[lin(tm,lambda m: acc[j,m*7+k,r:r+8,:]) for k in range(7)]
                        for k in range(4):
                            y=lin(WT[k],lambda m: ps[m])
                            out[k^fl]=y if out[k^fl] is None else out[k^fl]+y
                    return [out[:2],out[2:]]
                c=[rows(r0),rows(r0+8)]
                ys=[]
                for a in range(2):
                    for b in range(2):
                        rr=(2*(Q//2)+a)*SQ+r0; cc=(2*(Q%2)+b)*128
                        ys.append(pk2(c[0][a][b],c[1][a][b])); ob[j,rr:rr+16,cc:cc+128]=up(ys[-1])
                return ys
            return [(lambda r0=r0,Q=Q: job(r0,Q)) for r0 in range(0,SQ,16) for Q in range(4)]
        def half(par,j,never,dq=True,da=True,do=True,wq=True,wo=True,first=False,extra=(),cnt0=0):
            pend=[]
            def tie(vs_):
                vs_=list(vs_)
                for t in range(1,len(vs_)):
                    if pend: vs_[t]=jnp.where(never,pend.pop(0),vs_[t])
                return up(jnp.concatenate(vs_,axis=0))
            items=[]; jobs=list(extra)
            def add(fs,n,lo,hi):
                for t,f in enumerate(fs): items.append((lo+(hi-lo)*(t+0.5)/len(fs),len(items),n,f))
            unit=lambda Q,k: (2*(Q//2)+k//2)*4+2*(Q%2)+k%2
            if da:
                sl=par; e=[None]*16
                def qk(Q,k):
                    u=unit(Q,k)
                    cs=[lin(WT[Q],lambda i: qc[par,j,i*4+k,r:r+8,:]) for r in range(0,SQ,8)]
                    q=up(jnp.concatenate([pk2(cs[t],cs[t+1]) for t in range(0,10,2)],axis=0))
                    sc=jax.lax.dot_general(tile(ks,sl,j,u),q,NT,preferred_element_type=F32)
                    z=jnp.exp2((sc-jnp.max(sc,axis=0,keepdims=True))*C2)
                    l=jnp.sum(z,axis=0,keepdims=True)
                    y=pl.reciprocal(l,approx=True); r=y*(2.0-l*y)
                    e[u]=(z*r).astype(BF16).T
                def pv(k):
                    o=[jnp.dot(e[unit(Q,k)],tile(vs,sl,j,unit(Q,k)),preferred_element_type=F32) for Q in range(4)]
                    for i in range(7): os_[par,j,i*4+k]=lin(LT[i],lambda Q: o[Q])
                k0,k1,lg=(*T_QK,T_PV) if (dq and do) else (*T_QK_SHORT,T_PV_SHORT)
                add([(lambda Q=Q,k=k: qk(Q,k)) for k in range(4) for Q in QO],1,k0,k1)
                add([(lambda k=k: pv(k)) for k in range(4)],4,k0+lg,k1+lg)
            if dq:
                slq,jq=1-par,j; tmp={}
                def qd(p): return jnp.dot(tie([xc[jq,p,t:t+8,:] for t in range(0,SQ//2,8)]),up(wqc[slq,p]),preferred_element_type=F32)
                def q3(i,m): tmp[i,m]=qd(i*7+m)
                def q4(i):
                    ms={m:qd(i*7+m) for m in (0,3,4,6)}
                    for k in range(4): qc[1-par,j,i*4+(k^FLIP[i])]=lin(WT[k],lambda m: ms[m] if m in ms else tmp[i,m])
                w=(T_QP[1]-T_QP[0])/7
                for i in range(7):
                    add([(lambda m=m,i=i: q3(i,m)) for m in (1,2,5)],1,T_QP[0]+w*(i-T_QLEAD),T_QP[0]+w*(i+0.6-T_QLEAD))
                    add([lambda i=i: q4(i)],4,T_QP[0]+w*(i+0.8),T_QP[0]+w*(i+0.8))
                if wq: jobs+=w_jobs(wqs,wqc,1-slq,jq)
            if do:
                slo,jo=1-par,j
                def od(p):
                    cs=[lin(LT[p%7],lambda k: os_[1-par,j,(p//7)*4+k,t:t+8,:]) for t in range(0,SQ,8)]
                    y=jnp.dot(tie([pk2(cs[t],cs[t+1]) for t in range(0,10,2)]),up(woc[slo,p]),preferred_element_type=F32)
                    if first: acc[jo,p]=y
                    else: acc[jo,p]+=y
                add([(lambda p=p: od(p)) for p in range(R)],1,*T_OP)
                if wo: jobs+=w_jobs(wos,woc,1-slo,jo)
            if jobs: add([(lambda f=f: pend.extend(f())) for f in jobs],0,*T_JOB)
            cnt=cnt0; held=[]
            for _,_,n,f in sorted(items,key=lambda z:z[:2]):
                if n==4: held.append(f)
                else: f(); cnt+=n
                while held and cnt%4==0: held.pop(0)(); cnt+=4
            for f in held: f(); cnt+=4
            return cnt
        def run(jobs):
            for f in jobs: f()
        x_copy(0,0).start(); start_w(wq_copy,0,0)
        x_copy(0,0).wait()
        x_copy(0,1).start(); x_copy(0,2).start()
        run(x_jobs(0,0))
        wait_w(wq_copy,0,0)
        x_copy(0,3).start(); start_w(wq_copy,1,1); start_kv0(0)
        full_w(wqs,wqc,0)
        start_w(wq_copy,2,0); start_w(wo_copy,0,0)
        @pl.loop(0,NJ)
        def _(j):
            half(1,j,j<0,da=False,do=False,wq=False)
            @pl.when(j<NJ-1)
            def _():
                x_copy(0,j+1).wait(); start_kv0(j+1); run(x_jobs(0,j+1))
        start_kv(1,1,(0,))
        wait_w(wq_copy,1,1); full_w(wqs,wqc,1)
        wait_w(wq_copy,2,0); wait_w(wo_copy,0,0)
        def quad(par,never,extra=lambda j: (),pre=None,post=None,**kw):
            c=0
            for j in range(NJ):
                if pre: pre(j)
                c=half(par,j,never,extra=extra(j),cnt0=c,**kw)
                if post: post(j)
        @pl.loop(0,NGG+1)
        def _(g):
            never=g<0
            @pl.when(g==0)
            def _():
                start_w(wq_copy,3,1); start_w(wo_copy,1,1)
                def pre(j):
                    wait_kv0(j)
                    if j==0: start_kv(1,1,(1,))
                quad(0,never,extra=lambda j: w_jobs(wos,woc,0,j),pre=pre,do=False)
            @pl.when(g==3)
            def _():
                for j in range(NJ): x_copy(1,j).start()
            @pl.when(g==NG-2)
            def _():
                for j in range(NJ): x_copy(1,j).wait()
            @pl.when(g==NG-1)
            def _():
                pl.loop(0,NJ)(lambda j: run(x_jobs(1,j)))
            @pl.when(g==NG+1)
            def _():
                pl.loop(0,NJ)(lambda j: run(fin_jobs(j)))
            for par,first in ((0,False),(1,True),(1,False)):
                cond=(g%2==par)&(g>0)&(g<NGG-1)
                if par: cond=cond&((g%NG==1) if first else (g%NG!=1))
                @pl.when(cond)
                def _():
                    wait_w(wq_copy,g+2,par); wait_w(wo_copy,g,par); wait_kv(par,(0,) if first else (0,1))
                    def post(j):
                        if j==0: start_w(wq_copy,g+3,1-par); start_w(wo_copy,g+1,1-par); start_kv(g+1,1-par)
                    quad(par,never,first=first,pre=lambda j: wait_kv(par,(1,)) if (first and j==CUT) else None,post=post)
            @pl.when(g==NG+1)
            def _():
                for j in range(NJ): o_copy(0,j).start()
            @pl.when(g==NG+2)
            def _():
                for j in range(NJ): o_copy(0,j).wait()
            @pl.when(g==NGG-1)
            def _():
                wait_w(wo_copy,NGG-1,1); wait_kv(1)
                quad(1,never,dq=False)
            @pl.when(g==NGG)
            def _():
                quad(0,never,dq=False,da=False,wo=False,extra=lambda j: fin_jobs(j-1) if j else (),post=lambda j: o_copy(1,j-1).start() if j else None)
                run(fin_jobs(NJ-1)); o_copy(1,NJ-1).start()
        for j in range(NJ): o_copy(1,j).wait()

    def f(ax,ak,av,awq,awo,bx,bk,bv,bwq,bwo):
        V=pltpu.VMEM; S=pltpu.SemaphoreType.DMA
        out=pl.pallas_call(kern,grid=(1,),in_specs=[pl.BlockSpec(memory_space=pl.ANY)]*10,
            out_specs=pl.BlockSpec(memory_space=pl.ANY),
            out_shape=jax.ShapeDtypeStruct((B*SQ,2*D),BF16),
            scratch_shapes=[V((2,NJ,MS,D),BF16),V((NJ,R,SQ//2,128),U32),V((2,512,512),BF16),V((2,512,512),BF16),
                V((2,R,64,128),U32),V((2,R,64,128),U32),
                V((2,B,NH,SK,DH),BF16),V((2,B,NH,SK,DH),BF16),
                V((2,NJ,28,SQ,128),F32),V((2,NJ,28,SQ,DH),F32),V((NJ,R,SQ,128),F32),V((NJ,MS,D),BF16),
                S((2*NJ,)),S((2,)),S((2,)),S((8,)),S((2*NJ,)),S((NJ,))],
            compiler_params=pltpu.CompilerParams(vmem_limit_bytes=100*2**20),
        )(ax.reshape(B*SQ,D),ak,av,awq,awo,bx.reshape(B*SQ,D),bk,bv,bwq,bwo)
        return out.reshape(B,SQ,2*D)
    return f


@jax.jit
def pallas_concat_heads__mha_block_cached__mha_block_cached__near_ridge_kernel(
    A_x, A_k_cache, A_v_cache, A_wq, A_wo, B_x, B_k_cache, B_v_cache, B_wq, B_wo):
    return build()(A_x, A_k_cache, A_v_cache, A_wq, A_wo, B_x, B_k_cache, B_v_cache, B_wq, B_wo)
```
